```python
import jax
import jax.numpy as jnp

def _softmax(x, axis=-1):
    return jax.nn.softmax(x, axis=axis)

def _gelu(x):
    return jax.nn.gelu(x, approximate=True)

def _silu(x):
    return jax.nn.silu(x)

def _sigmoid(x):
    return jax.nn.sigmoid(x)

def _layernorm(x, axis=-1, eps=1e-05):
    m = jnp.mean(x, axis=axis, keepdims=True)
    v = jnp.var(x, axis=axis, keepdims=True)
    return (x - m) / jnp.sqrt(v + eps)

def _scatter_add(tgt, idx, src, axis=0):
    return tgt.at[idx].add(src)

def _segment_sum(src, seg, n):
    return jax.ops.segment_sum(src, seg, n)

class _Rng:

    def __init__(self, key):
        self._k = key

    def _next(self):
        self._k, sub = jax.random.split(self._k)
        return sub

    def normal(self, shape):
        return jax.random.normal(self._next(), shape, dtype=jnp.bfloat16)

    def randint(self, lo, hi, shape):
        return jax.random.randint(self._next(), shape, lo, hi, dtype=jnp.int32)

    def uniform(self, shape, lo=0.0, hi=1.0):
        return jax.random.uniform(self._next(), shape, jnp.bfloat16, lo, hi)

    def permutation(self, n):
        return jax.random.permutation(self._next(), n)
kernel_name = 'adaLN_cond__memory_aug_recurrent_mem_tr__moe_arch_mod__prompt'

def setup_inputs():
    _rng = _Rng(jax.random.key(int.from_bytes(__import__("os").urandom(4), "little")))
    _w = lambda a: (lambda t: t.astype(jnp.bfloat16) if jnp.issubdtype(t.dtype, jnp.floating) else t)(jnp.asarray(a))

    def _A_setup():
        B, S, Dm = (1, 2048, 1024)
        H, Dh = (32, 128)
        M, seg = (8, 32)
        seg = min(seg, S)
        S = S // seg * seg
        return {'x': _w((lambda *s: _rng.normal(s) * 0.05)(B, S, Dm)), 'mem0': _w((lambda *s: _rng.normal(s) * 0.05)(B, M, Dm)), 'Wq': _w((lambda *s: _rng.normal(s) * 0.05)(Dm, H, Dh) * Dm ** (-0.5)), 'Wk': _w((lambda *s: _rng.normal(s) * 0.05)(Dm, H, Dh) * Dm ** (-0.5)), 'Wv': _w((lambda *s: _rng.normal(s) * 0.05)(Dm, H, Dh) * Dm ** (-0.5)), 'Wo': _w((lambda *s: _rng.normal(s) * 0.05)(H, Dh, Dm) * (H * Dh) ** (-0.5)), 'seg_len': seg}
    _A_in = _A_setup()

    def _B_setup():
        B, S, D, F, C = (1, 2048, 1024, 3584, 2)
        return {'x': _w((lambda *s: _rng.normal(s) * 0.05)(B, S, D)), 'w_r': _w((lambda *s: _rng.normal(s) * 0.05)(D)), 'w_gate': _w((lambda *s: _rng.normal(s) * 0.05)(D, F)), 'w_up': _w((lambda *s: _rng.normal(s) * 0.05)(D, F)), 'w_down': _w((lambda *s: _rng.normal(s) * 0.05)(F, D))}
    _B_in = _B_setup()
    return {'A_x': _A_in['x'], 'A_mem0': _A_in['mem0'], 'A_Wq': _A_in['Wq'], 'A_Wk': _A_in['Wk'], 'A_Wv': _A_in['Wv'], 'A_Wo': _A_in['Wo'], 'A_seg_len': _A_in['seg_len'], 'B_x': _B_in['x'], 'B_w_r': _B_in['w_r'], 'B_w_gate': _B_in['w_gate'], 'B_w_up': _B_in['w_up'], 'B_w_down': _B_in['w_down'], 'c': _w((lambda *s: _rng.normal(s) * 0.05)(1, 1024)), 'w_mod': _w((lambda *s: _rng.normal(s) * 0.05)(1024, 6 * 1024) * 1024 ** (-0.5))}

def reference(A_x, A_mem0, A_Wq, A_Wk, A_Wv, A_Wo, A_seg_len, B_x, B_w_r, B_w_gate, B_w_up, B_w_down, c, w_mod):

    def _A_ref(x, mem0, Wq, Wk, Wv, Wo, seg_len):
        B, S, Dm = x.shape
        H, Dh = (Wq.shape[1], Wq.shape[2])
        M = mem0.shape[1]
        scale = Dh ** (-0.5)
        n_seg = S // seg_len
        L = M + seg_len
        idx = jnp.arange(L)
        mask = (idx[:, None] < M) | (idx[:, None] >= idx[None, :])
        mem = mem0
        outs = []
        for s in range(n_seg):
            xs = x[:, s * seg_len:(s + 1) * seg_len, :].copy()
            h = jnp.concatenate([mem, xs], axis=1)
            q = jnp.einsum('btd,dhe->bhte', h, Wq)
            k = jnp.einsum('btd,dhe->bhte', h, Wk)
            v = jnp.einsum('btd,dhe->bhte', h, Wv)
            scores = jnp.einsum('bhqe,bhke->bhqk', q, k) * scale
            scores = jnp.where(mask[None, None], scores, -1000000000.0)
            p = _softmax(scores, axis=-1)
            o = jnp.einsum('bhqk,bhke->bhqe', p, v)
            o = jnp.einsum('bhte,hed->btd', o, Wo)
            mem = o[:, :M, :].copy()
            outs.append(o[:, M:, :])
        return jnp.concatenate(outs, axis=1)

    def _B_ref(x, w_r, w_gate, w_up, w_down):
        B, S, D = x.shape
        C = 2
        r = x @ w_r
        idx = jnp.argsort(-r, axis=-1)[:, :C]
        idx_e = jnp.repeat(idx.reshape(B, C, 1), D, axis=2)
        x_sel = jnp.take_along_axis(x, idx_e, axis=1)
        g = _silu(x_sel @ w_gate)
        u = x_sel @ w_up
        y = g * u @ w_down
        r_sel = _sigmoid(jnp.take_along_axis(r, idx, axis=1))
        y = y * r_sel.reshape(B, C, 1)
        b_off = (jnp.arange(B) * S).reshape(B, 1)
        flat_idx = (idx + b_off).reshape(B * C)
        zero = (x * 0.0).reshape(B * S, D)
        upd = _scatter_add(zero, flat_idx, y.reshape(B * C, D), axis=0)
        return x + upd.reshape(B, S, D)
    x = A_x
    mod = (_silu(c) @ w_mod).reshape(c.shape[0], 6, 1, -1)
    sa, ca, ga, sb, cb, gb = (mod[:, 0].copy(), mod[:, 1].copy(), mod[:, 2].copy(), mod[:, 3].copy(), mod[:, 4].copy(), mod[:, 5].copy())
    h = _layernorm(x, axis=-1) * (1 + ca) + sa
    x = x + ga * _A_ref(h, A_mem0, A_Wq, A_Wk, A_Wv, A_Wo, A_seg_len)
    h = _layernorm(x, axis=-1) * (1 + cb) + sb
    x = x + gb * _B_ref(h, B_w_r, B_w_gate, B_w_up, B_w_down)
    return x
```

```python
import functools

import jax
import jax.numpy as jnp
from jax import lax
import jax.experimental.pallas as pl
import jax.experimental.pallas.tpu as pltpu

BF = jnp.bfloat16
F32 = jnp.float32

S = 2048
D = 1024
H = 32
DH = 128
NM = 8
SEG = 32
NSEG = S // SEG
F = 3584
R0 = 512
XR = 24
RING = 576
QOFF = 64
EPS = 1e-5
NEG = -1000000000.0


def _dot(a, b):
    return jnp.dot(a, b, preferred_element_type=F32)


def _dot_t(a, b):
    return lax.dot_general(a, b, (((1,), (1,)), ((), ())),
                           preferred_element_type=F32)


def _ln(xf):
    m = jnp.mean(xf, axis=-1, keepdims=True)
    d = xf - m
    v = jnp.mean(d * d, axis=-1, keepdims=True)
    return d * lax.rsqrt(v + EPS)


def _kernel(c_ref, wr_ref, mem0_ref, x_hbm, wq_hbm, wk_hbm, wv_hbm, wo_hbm,
            wg_hbm, wu_hbm, wd_hbm, wmod_hbm, out_hbm,
            w_all, wo_all, x_buf, h_buf, ring, oring, out_buf, r_buf, mod_buf,
            sems):
    w_hbm = (wq_hbm, wk_hbm, wv_hbm)
    scale = DH ** (-0.5)

    cp_x0 = pltpu.make_async_copy(x_hbm.at[0, pl.ds(0, R0)],
                                  x_buf.at[pl.ds(0, R0)], sems.at[0])
    cp_x1 = pltpu.make_async_copy(x_hbm.at[0, pl.ds(R0, S - R0)],
                                  x_buf.at[pl.ds(R0, S - R0)], sems.at[1])
    cp_wo = [pltpu.make_async_copy(wo_hbm.at[:, pl.ds(n * 128, 128)],
                                   wo_all.at[n], sems.at[2])
             for n in range(D // 128)]

    def prologue(wm_buf, stage, tmp, acc, psem):
        cp_m0 = pltpu.make_async_copy(wmod_hbm.at[:, pl.ds(0, 2 * D)],
                                      wm_buf.at[:, pl.ds(0, 2 * D)], psem.at[3])
        cp_m1 = pltpu.make_async_copy(wmod_hbm.at[:, pl.ds(2 * D, 4 * D)],
                                      wm_buf.at[:, pl.ds(2 * D, 4 * D)],
                                      psem.at[4])

        def chunk_copy(w, kc, slot):
            return pltpu.make_async_copy(
                w_hbm[w].at[pl.ds(kc * 128, 128)], stage.at[slot],
                psem.at[slot])

        cp_m0.start()
        cp_x0.start()
        chunk_copy(0, 0, 0).start()
        chunk_copy(0, 1, 1).start()
        cp_x1.start()

        cf = c_ref[...].astype(F32)
        sc = (cf * jax.nn.sigmoid(cf)).astype(BF)
        sc16 = jnp.broadcast_to(sc, (16, D))

        def mod_cols(lo, hi):
            for j in range(lo, hi):
                m = _dot(sc16, wm_buf[:, j * D:(j + 1) * D])
                mod_buf[j] = m[0:8].astype(BF).astype(F32)

        cp_m0.wait()
        mod_cols(0, 2)
        sa = mod_buf[0][0:1]
        ca1 = 1.0 + mod_buf[1][0:1]

        def ln_rows(i, _):
            r = pl.multiple_of(i * 64, 64)
            xf = x_buf[pl.ds(r, 64), :].astype(F32)
            h_buf[pl.ds(r, 64), :] = (_ln(xf) * ca1 + sa).astype(BF)
            return 0

        cp_x0.wait()
        lax.fori_loop(0, R0 // 64, ln_rows, 0)

        def relayout(w, kc, slot):
            for dc in range(8):
                v = stage[slot, pl.ds(dc * 16, 16)]
                u = pltpu.bitcast(v, jnp.uint32)
                tmp[pl.ds(dc * 256, 256), :] = u.reshape(256, 128)
            k0 = kc * 64
            for hp in range(H // 2):
                a = tmp[pl.ds(hp, 128, stride=H // 2), :]
                lo = pltpu.bitcast(a << 16, F32).astype(BF)
                hi = pltpu.bitcast(a & jnp.uint32(0xFFFF0000), F32).astype(BF)
                w_all[w * H + 2 * hp, pl.ds(k0, 64), :] = pltpu.bitcast(lo, jnp.uint32)
                w_all[w * H + 2 * hp + 1, pl.ds(k0, 64), :] = pltpu.bitcast(hi, jnp.uint32)

        def project(w, kc, mode):
            k0 = pl.multiple_of(kc * 128, 128)
            lhs = h_buf[pl.ds(0, R0), pl.ds(k0, 128)]

            def one(h, _):
                y = _dot(lhs, pltpu.bitcast(w_all[w * H + h, pl.ds(kc * 64, 64), :], BF))
                if mode == 0:
                    acc[h] = y
                elif mode == 1:
                    acc[h] += y
                else:
                    ring[w * H + h, pl.ds(QOFF, R0), :] = (acc[h] + y).astype(BF)
                return 0

            lax.fori_loop(0, H, one, 0, unroll=8)

        nchunk = 8 * 3
        for ci in range(nchunk):
            w, kc = divmod(ci, 8)
            slot = ci % 3
            if ci + 2 < nchunk:
                w2, kc2 = divmod(ci + 2, 8)
                chunk_copy(w2, kc2, (ci + 2) % 3).start()
            if ci == 4:
                cp_m1.start()
            if ci == 10:
                for cp in cp_wo:
                    cp.start()
            chunk_copy(w, kc, slot).wait()
            relayout(w, kc, slot)
            project(w, kc, 0 if kc == 0 else (2 if kc == 7 else 1))
            if ci == 7:
                cp_x1.wait()
                lax.fori_loop(R0 // 64, S // 64, ln_rows, 0)

        cp_m1.wait()
        mod_cols(2, 6)
        for cp in cp_wo:
            cp.wait()

    pl.run_scoped(
        prologue,
        pltpu.VMEM((D, 6 * D), BF),
        pltpu.VMEM((3, 128, H, DH), BF),
        pltpu.VMEM((128 * H // 2, 128), jnp.uint32),
        pltpu.VMEM((H, R0, 128), F32),
        pltpu.SemaphoreType.DMA((5,)),
    )

    def main(wg, wu, wd, fsem, acc_o):
        wo_u32 = wo_all.bitcast(jnp.uint32)
        ffn_copies = []
        for n in range(F // 128):
            ffn_copies.append(pltpu.make_async_copy(
                wg_hbm.at[:, pl.ds(n * 128, 128)], wg.at[n], fsem.at[0]))
            ffn_copies.append(pltpu.make_async_copy(
                wu_hbm.at[:, pl.ds(n * 128, 128)], wu.at[n], fsem.at[1]))
        for n in range(D // 128):
            ffn_copies.append(pltpu.make_async_copy(
                wd_hbm.at[:, pl.ds(n * 128, 128)], wd.at[n], fsem.at[2]))
        for cp in ffn_copies:
            cp.start()

        ga = mod_buf[2][0:1]
        sb = mod_buf[3][0:1]
        cb1 = 1.0 + mod_buf[4][0:1]
        gb = mod_buf[5][0:1]
        wr = wr_ref[...].astype(F32).reshape(1, D)

        def finish_rows(att, r, n):
            rows = pl.ds(r, n)
            x2 = (x_buf[rows, :].astype(F32)
                  + ga * att.astype(BF).astype(F32)).astype(BF)
            x_buf[rows, :] = x2
            x2f = x2.astype(F32)
            h2 = (_ln(x2f) * cb1 + sb).astype(BF).astype(F32)
            out_buf[rows, :] = (x2f + gb * h2).astype(BF)
            rr = jnp.sum(h2 * wr, axis=-1, keepdims=True)
            rr = rr.astype(BF).astype(F32)
            r_buf[rows, :] = jnp.broadcast_to(rr, (n, 128))

        def attn_mask(par):
            qi = lax.broadcasted_iota(jnp.int32, (48, 48), 0)
            ki = lax.broadcasted_iota(jnp.int32, (48, 48), 1)
            mlo = 40 if par == 0 else 32
            kmem = (ki >= mlo) & (ki < mlo + NM)
            kx = ki < SEG
            return kmem | (kx & ((qi >= SEG) | (qi >= ki)))

        def step(mem, j, par):
            s = 2 * j + par
            xr = pl.multiple_of(R0 + 48 * j + XR * par, 8)
            hx = h_buf[pl.ds(xr, XR), :]
            lhs = (jnp.concatenate([hx, mem], axis=0) if par == 0
                   else jnp.concatenate([mem, hx], axis=0))
            wbase = lax.rem(R0 + QOFF + 48 * j, RING)
            wpos = pl.multiple_of(wbase + XR * par, 8)
            spos = pl.multiple_of(lax.rem(SEG * s + QOFF, RING), SEG)
            opos = pl.multiple_of(lax.rem(SEG * s, RING), SEG)
            obase = lax.rem(48 * j, RING)
            rpos = pl.multiple_of(obase + XR * par, 8)
            mask = attn_mask(par)
            mrow = (slice(40, 48) if par == 0 else slice(32, 40))

            G = 4
            NG = H // G
            st = {}

            def proj(g, w):
                for h in range(g * G, (g + 1) * G):
                    y = _dot(lhs, pltpu.bitcast(w_all[w * H + h], BF)).astype(BF)
                    if par == 0:
                        ring[w * H + h, pl.ds(wpos, XR), :] = y[0:24]
                        st[w, h] = y[16:32]
                    else:
                        ring[w * H + h, pl.ds(wpos, XR), :] = y[8:32]
                        st[w, h] = y[0:16]

            def seg(w, h):
                return jnp.concatenate(
                    [ring[w * H + h, pl.ds(spos, SEG), :], st[w, h]], axis=0)

            def qk(g):
                for h in range(g * G, (g + 1) * G):
                    sc = _dot_t(seg(0, h), seg(1, h)) * scale
                    sc = jnp.where(mask, sc, NEG)
                    mx = jnp.max(sc, axis=-1, keepdims=True)
                    e = jnp.exp(sc - mx)
                    p = e / jnp.sum(e, axis=-1, keepdims=True)
                    st['p', h] = p.astype(BF)

            def pv(g):
                for h in range(g * G, (g + 1) * G):
                    o = _dot(st['p', h], seg(2, h)).astype(BF)
                    oring[h, pl.ds(opos, SEG), :] = o[0:SEG]
                    if par == 0:
                        lo = jnp.concatenate(
                            [oring[h, pl.ds(rpos, XR), :], o[mrow]], axis=0)
                    else:
                        lo = jnp.concatenate(
                            [o[mrow], oring[h, pl.ds(rpos, XR), :]], axis=0)
                    st['o', h] = lo

            def wo(g):
                lo = jnp.concatenate(
                    [st['o', h] for h in range(g * G, (g + 1) * G)], axis=1)
                for n in range(D // 128):
                    wt = wo_u32[n, pl.ds(g * G * 64, G * 64), :]
                    y = _dot(lo, pltpu.bitcast(wt, BF))
                    if g == 0:
                        acc_o[n] = y
                    elif g < NG - 1:
                        acc_o[n] += y
                    else:
                        st['a', n] = acc_o[n] + y

            for g in range(NG + 2):
                if 1 <= g <= NG:
                    qk(g - 1)
                if g < NG:
                    proj(g, 0)
                    proj(g, 1)
                if 1 <= g <= NG:
                    pv(g - 1)
                if g < NG:
                    proj(g, 2)
                if 2 <= g:
                    wo(g - 2)
            acc = jnp.concatenate([st['a', n] for n in range(D // 128)], axis=1)
            if par == 0:
                att, mem_new = acc[0:24], acc[24:32]
            else:
                att, mem_new = acc[8:32], acc[0:8]
            finish_rows(att, pl.multiple_of(48 * j + XR * par, 8), XR)
            return mem_new.astype(BF)

        def dstep(j, mem):
            mem = step(mem, j, 0)
            return step(mem, j, 1)

        lax.fori_loop(0, NSEG // 2, dstep, mem0_ref[0])

        done = XR * NSEG
        cp_o0 = pltpu.make_async_copy(out_buf.at[pl.ds(0, done)],
                                      out_hbm.at[0, pl.ds(0, done)], fsem.at[3])
        cp_o0.start()

        def tail_rows(b, _):
            r = pl.multiple_of(done + 64 * b, 64)
            pos = pl.multiple_of(lax.rem(r, RING), 64)
            lo = jnp.concatenate(
                [oring[h, pl.ds(pos, 64), :] for h in range(H)], axis=1)
            att = jnp.concatenate(
                [_dot(lo, wo_all[n]) for n in range(D // 128)], axis=1)
            finish_rows(att, r, 64)
            return 0

        lax.fori_loop(0, (S - done) // 64, tail_rows, 0)

        ridx = lax.broadcasted_iota(jnp.int32, (S, 128), 0)
        rv = r_buf[...]
        m1 = jnp.max(rv)
        i1 = jnp.min(jnp.where(rv == m1, ridx, S))
        rv2 = jnp.where(ridx == i1, -jnp.inf, rv)
        m2 = jnp.max(rv2)
        i2 = jnp.min(jnp.where((rv2 == m2) & (ridx != i1), ridx, S))
        i1 = jnp.clip(i1, 0, S - 1)
        i2 = jnp.clip(i2, 0, S - 1)

        slab_i = lax.broadcasted_iota(jnp.int32, (16, D), 0)

        def get_row(i):
            b = pl.multiple_of((i // 16) * 16, 16)
            slab = x_buf[pl.ds(b, 16), :].astype(F32)
            return jnp.sum(jnp.where(slab_i == i - b, slab, 0.0), axis=0,
                           keepdims=True)

        x2s = jnp.where(slab_i == 0, get_row(i1),
                        jnp.where(slab_i == 1, get_row(i2), 0.0))
        h2s = (_ln(x2s) * cb1 + sb).astype(BF)

        for cp in ffn_copies:
            cp.wait()
        gu = []
        for n in range(F // 128):
            g = _dot(h2s, wg[n]).astype(BF).astype(F32)
            u = _dot(h2s, wu[n]).astype(BF).astype(F32)
            g = (g * jax.nn.sigmoid(g)).astype(BF).astype(F32)
            gu.append((g * u).astype(BF))
        gu = jnp.concatenate(gu, axis=1)
        y = jnp.concatenate([_dot(gu, wd[n]) for n in range(D // 128)], axis=1)
        rsel = jnp.where(slab_i[:, 0:1] == 0, m1, m2)
        y = y.astype(BF).astype(F32) * jax.nn.sigmoid(rsel)
        fixed = x2s + gb * (h2s.astype(F32) + y.astype(BF).astype(F32))

        cp_o0.wait()

        def put_row(i, row):
            b = pl.multiple_of((i // 16) * 16, 16)
            slab = out_buf[pl.ds(b, 16), :].astype(F32)
            out_buf[pl.ds(b, 16), :] = jnp.where(
                slab_i == i - b, row, slab).astype(BF)
            return b

        b1 = put_row(i1, fixed[0:1])
        b2 = put_row(i2, fixed[1:2])
        cp_o1 = pltpu.make_async_copy(out_buf.at[pl.ds(done, S - done)],
                                      out_hbm.at[0, pl.ds(done, S - done)],
                                      fsem.at[3])
        cp_o1.start()
        cp_o1.wait()
        for b in (b1, b2):
            cp = pltpu.make_async_copy(out_buf.at[pl.ds(b, 16)],
                                       out_hbm.at[0, pl.ds(b, 16)], fsem.at[3])
            cp.start()
            cp.wait()

    pl.run_scoped(
        main,
        pltpu.VMEM((F // 128, D, 128), BF),
        pltpu.VMEM((F // 128, D, 128), BF),
        pltpu.VMEM((D // 128, F, 128), BF),
        pltpu.SemaphoreType.DMA((4,)),
        pltpu.VMEM((D // 128, 32, 128), F32),
    )


@functools.partial(jax.jit, static_argnames=("A_seg_len",))
def pallas_adaLN_cond__memory_aug_recurrent_mem_tr__moe_arch_mod__prompt_kernel(
    A_x: jax.Array,
    A_mem0: jax.Array,
    A_Wq: jax.Array,
    A_Wk: jax.Array,
    A_Wv: jax.Array,
    A_Wo: jax.Array,
    A_seg_len: int,
    B_x: jax.Array,
    B_w_r: jax.Array,
    B_w_gate: jax.Array,
    B_w_up: jax.Array,
    B_w_down: jax.Array,
    c: jax.Array,
    w_mod: jax.Array,
):
    assert int(A_seg_len) == SEG
    assert A_x.shape == (1, S, D) and A_Wq.shape == (D, H, DH)
    vm = pl.BlockSpec(memory_space=pltpu.VMEM)
    hbm = pl.BlockSpec(memory_space=pl.ANY)
    return pl.pallas_call(
        _kernel,
        out_shape=jax.ShapeDtypeStruct((1, S, D), BF),
        in_specs=[vm, vm, vm] + [hbm] * 9,
        out_specs=hbm,
        scratch_shapes=[
            pltpu.VMEM((3 * H, D // 2, DH), jnp.uint32),
            pltpu.VMEM((D // 128, H * DH, 128), BF),
            pltpu.VMEM((S, D), BF),
            pltpu.VMEM((S, D), BF),
            pltpu.VMEM((3 * H, RING, DH), BF),
            pltpu.VMEM((H, RING, DH), BF),
            pltpu.VMEM((S, D), BF),
            pltpu.VMEM((S, 128), F32),
            pltpu.VMEM((6, 8, D), F32),
            pltpu.SemaphoreType.DMA((3,)),
        ],
        compiler_params=pltpu.CompilerParams(
            vmem_limit_bytes=120 * 1024 * 1024),
    )(c, B_w_r, A_mem0, A_x, A_Wq, A_Wk, A_Wv,
      A_Wo.reshape(H * DH, D), B_w_gate, B_w_up, B_w_down, w_mod)
```

```python
import functools

import jax
import jax.numpy as jnp
from jax import lax
import jax.experimental.pallas as pl
import jax.experimental.pallas.tpu as pltpu

BF = jnp.bfloat16
F32 = jnp.float32

S = 2048
D = 1024
H = 32
DH = 128
NM = 8
SEG = 32
NSEG = S // SEG
F = 3584
R0 = 512
XR = 24
RING = 576
QOFF = 64
EPS = 1e-5
NEG = -1000000000.0
KC = 256
NKC = D // KC


def _dot(a, b):
    return jnp.dot(a, b, preferred_element_type=F32)


def _dot_t(a, b):
    return lax.dot_general(a, b, (((1,), (1,)), ((), ())),
                           preferred_element_type=F32)


def _ln(xf):
    m = jnp.mean(xf, axis=-1, keepdims=True)
    d = xf - m
    v = jnp.mean(d * d, axis=-1, keepdims=True)
    return d * lax.rsqrt(v + EPS)


def _kernel(c_ref, wr_ref, mem0_ref, x_hbm, wq_hbm, wk_hbm, wv_hbm, wo_hbm,
            wg_hbm, wu_hbm, wd_hbm, wmod_hbm, out_hbm,
            w_all, wo_all, x_buf, h_buf, ring_q, ring_k, ring_v, oring, out_buf, r_buf, mod_buf,
            sems):
    w_hbm = (wq_hbm, wk_hbm, wv_hbm)
    ring = (ring_q, ring_k, ring_v)
    scale = DH ** (-0.5)

    cp_x0 = pltpu.make_async_copy(x_hbm.at[0, pl.ds(0, R0)],
                                  x_buf.at[pl.ds(0, R0)], sems.at[0])
    cp_x1 = pltpu.make_async_copy(x_hbm.at[0, pl.ds(R0, S - R0)],
                                  x_buf.at[pl.ds(R0, S - R0)], sems.at[1])

    def cp_wo(n):
        c0 = pl.multiple_of(n * 128, 128)
        return pltpu.make_async_copy(wo_hbm.at[:, pl.ds(c0, 128)],
                                     wo_all.at[n], sems.at[2])

    def prologue(wm_buf, stage, tmp, acc, psem):
        cp_m0 = pltpu.make_async_copy(wmod_hbm.at[:, pl.ds(0, 2 * D)],
                                      wm_buf.at[:, pl.ds(0, 2 * D)], psem.at[3])

        def cp_m1(n):
            c0 = pl.multiple_of(2 * D + n * 512, 512)
            return pltpu.make_async_copy(wmod_hbm.at[:, pl.ds(c0, 512)],
                                         wm_buf.at[:, pl.ds(c0, 512)], psem.at[4])

        def chunk_copy(w, kc, slot):
            return pltpu.make_async_copy(
                w_hbm[w].at[pl.ds(kc * KC, KC)], stage.at[slot],
                psem.at[slot])

        chunk_copy(0, 0, 0).start()
        cp_m0.start()
        cp_x0.start()

        cf = c_ref[...].astype(F32)
        sc = (cf * jax.nn.sigmoid(cf)).astype(BF)
        sc16 = jnp.broadcast_to(sc, (16, D))

        def mod_cols(lo, hi):
            for j in range(lo, hi):
                m = _dot(sc16, wm_buf[:, j * D:(j + 1) * D])
                mod_buf[j] = m[0:8].astype(BF).astype(F32)

        def ln_rows(r, n):
            r = pl.multiple_of(r, 16)
            xf = x_buf[pl.ds(r, n), :].astype(F32)
            h_buf[pl.ds(r, n), :] = (_ln(xf) * (1.0 + mod_buf[1][0:1]) + mod_buf[0][0:1]).astype(BF)

        def ln_loop(i, _):
            ln_rows(i * 64, 64)
            return 0

        def unpack_stage(slot):
            for dc in range(KC // 16):
                v = stage[slot, pl.ds(dc * 16, 16)]
                u = pltpu.bitcast(v, jnp.uint32)
                tmp[pl.ds(dc * 256, 256), :] = u.reshape(256, 128)

        def relayout_pair(w, kc, hp):
            k0 = pl.multiple_of(kc * (KC // 2), KC // 2)
            a = tmp[pl.ds(hp, KC, stride=H // 2), :]
            lo = pltpu.bitcast(a << 16, F32).astype(BF)
            hi = pltpu.bitcast(a & jnp.uint32(0xFFFF0000), F32).astype(BF)
            w_all[w * H + 2 * hp, pl.ds(k0, KC // 2), :] = pltpu.bitcast(lo, jnp.uint32)
            w_all[w * H + 2 * hp + 1, pl.ds(k0, KC // 2), :] = pltpu.bitcast(hi, jnp.uint32)

        nchunk = NKC * 3

        def start_chunk(ci):
            for w in range(3):
                @pl.when((ci >= NKC * w) & (ci < NKC * w + NKC))
                def _():
                    kc = pl.multiple_of((ci - NKC * w) * KC, KC)
                    pltpu.make_async_copy(
                        w_hbm[w].at[pl.ds(kc, KC)], stage.at[ci % 3],
                        psem.at[ci % 3]).start()

        def wait_chunk(ci):
            chunk_copy(0, 0, ci % 3).wait()

        wait_chunk(0)
        chunk_copy(0, 1, 1).start()
        unpack_stage(0)
        for hp in range(H // 2):
            relayout_pair(0, 0, hp)
        cp_m0.wait()
        mod_cols(0, 2)

        chunk_copy(0, 2, 2).start()
        cp_x1.start()
        cp_x0.wait()
        lax.fori_loop(0, R0 // 64, ln_loop, 0)

        LNR = (S - R0) // (nchunk - NKC)

        def chunk_body(ci, with_ln):
            w, kc = ci // NKC, ci % NKC
            cn = jnp.minimum(ci + 1, nchunk - 1)
            start_chunk(ci + 3)
            if with_ln:
                cp_m1(ci - NKC).start()
                cp_wo(ci - NKC).start()

            @pl.when(ci + 1 < nchunk)
            def _():
                wait_chunk(ci + 1)

            k0 = pl.multiple_of(kc * KC, KC)
            lhs = h_buf[pl.ds(0, R0), pl.ds(k0, KC)]
            kw = pl.multiple_of(kc * (KC // 2), KC // 2)
            first = kc == 0
            hp_next = 0
            for h in range(H):
                y = _dot(lhs, pltpu.bitcast(w_all[w * H + h, pl.ds(kw, KC // 2), :], BF))
                acc[h] = jnp.where(first, y, acc[h] + y)
                if h == 3:
                    unpack_stage(cn % 3)
                if h >= 8 and h % 3 != 0:
                    relayout_pair(cn // NKC, cn % NKC, hp_next)
                    hp_next += 1
                if with_ln and h == 4:
                    ln_rows(R0 + (ci - NKC) * LNR, LNR)

            for wi in range(3):
                @pl.when(ci == NKC * wi + NKC - 1)
                def _():
                    def cvt(h, _):
                        ring[wi][h, pl.ds(QOFF, R0), :] = acc[h].astype(BF)
                        return 0
                    lax.fori_loop(0, H, cvt, 0, unroll=4)
            return 0

        acc[...] = jnp.zeros_like(acc)
        lax.fori_loop(0, NKC, lambda ci, _: chunk_body(ci, False), 0)
        cp_x1.wait()
        lax.fori_loop(NKC, nchunk, lambda ci, _: chunk_body(ci, True), 0)

        for n in range(8):
            cp_m1(n).wait()
        mod_cols(2, 6)
        for n in range(8):
            cp_wo(n).wait()

    pl.run_scoped(
        prologue,
        pltpu.VMEM((D, 6 * D), BF),
        pltpu.VMEM((3, KC, H, DH), BF),
        pltpu.VMEM((KC * H // 2, 128), jnp.uint32),
        pltpu.VMEM((H, R0, 128), F32),
        pltpu.SemaphoreType.DMA((5,)),
    )

    def main(wg, wu, wd, fsem, acc_o, att_buf):
        wo_u32 = wo_all.bitcast(jnp.uint32)
        ffn_copies = []
        for n in range(F // 128):
            ffn_copies.append(pltpu.make_async_copy(
                wg_hbm.at[:, pl.ds(n * 128, 128)], wg.at[n], fsem.at[0]))
            ffn_copies.append(pltpu.make_async_copy(
                wu_hbm.at[:, pl.ds(n * 128, 128)], wu.at[n], fsem.at[1]))
        for n in range(D // 128):
            ffn_copies.append(pltpu.make_async_copy(
                wd_hbm.at[:, pl.ds(n * 128, 128)], wd.at[n], fsem.at[2]))
        for cp in ffn_copies:
            cp.start()

        ga = mod_buf[2][0:1]
        sb = mod_buf[3][0:1]
        cb1 = 1.0 + mod_buf[4][0:1]
        gb = mod_buf[5][0:1]
        wr = wr_ref[...].astype(F32).reshape(1, D)

        def finish_rows(att, r, n):
            rows = pl.ds(r, n)
            x2 = (x_buf[rows, :].astype(F32)
                  + ga * att.astype(BF).astype(F32)).astype(BF)
            x_buf[rows, :] = x2
            x2f = x2.astype(F32)
            h2 = (_ln(x2f) * cb1 + sb).astype(BF).astype(F32)
            out_buf[rows, :] = (x2f + gb * h2).astype(BF)
            rr = jnp.sum(h2 * wr, axis=-1, keepdims=True)
            rr = rr.astype(BF).astype(F32)
            r_buf[rows, :] = jnp.broadcast_to(rr, (n, 128))

        def attn_mask(par):
            qi = lax.broadcasted_iota(jnp.int32, (48, 48), 0)
            ki = lax.broadcasted_iota(jnp.int32, (48, 48), 1)
            mlo = 40 if par == 0 else 32
            kmem = (ki >= mlo) & (ki < mlo + NM)
            kx = ki < SEG
            return kmem | (kx & ((qi >= SEG) | (qi >= ki)))

        def step(mem, j, par):
            s = 2 * j + par
            xr = pl.multiple_of(R0 + 48 * j + XR * par, 8)
            hx = h_buf[pl.ds(xr, XR), :]
            lhs = (jnp.concatenate([hx, mem], axis=0) if par == 0
                   else jnp.concatenate([mem, hx], axis=0))
            wbase = lax.rem(R0 + QOFF + 48 * j, RING)
            wpos = pl.multiple_of(wbase + XR * par, 8)
            spos = pl.multiple_of(lax.rem(SEG * s + QOFF, RING), SEG)
            opos = pl.multiple_of(lax.rem(SEG * s, RING), SEG)
            obase = lax.rem(48 * j, RING)
            rpos = pl.multiple_of(obase + XR * par, 8)
            mask = attn_mask(par)
            mrow = (slice(40, 48) if par == 0 else slice(32, 40))

            G = 4
            NG = H // G
            st = {}

            def proj(g, w, lo=0, hi=G):
                for h in range(g * G + lo, g * G + hi):
                    y = _dot(lhs, pltpu.bitcast(w_all[w * H + h], BF)).astype(BF)
                    if par == 0:
                        ring[w][h, pl.ds(wpos, XR), :] = y[0:24]
                        st[w, h] = y[16:32]
                    else:
                        ring[w][h, pl.ds(wpos, XR), :] = y[8:32]
                        st[w, h] = y[0:16]

            def seg(w, h):
                return jnp.concatenate(
                    [ring[w][h, pl.ds(spos, SEG), :], st[w, h]], axis=0)

            def qk(g):
                for h in range(g * G, (g + 1) * G):
                    sc = _dot_t(seg(0, h), seg(1, h)) * scale
                    sc = jnp.where(mask, sc, NEG)
                    mx = jnp.max(sc, axis=-1, keepdims=True)
                    e = jnp.exp(sc - mx)
                    st['p', h] = e.astype(BF)
                    den = jnp.sum(e, axis=-1, keepdims=True)
                    r = pl.reciprocal(den, approx=True)
                    st['r', h] = r * (2.0 - den * r)

            def pv(g):
                for h in range(g * G, (g + 1) * G):
                    o = (_dot(st['p', h], seg(2, h)) * st['r', h]).astype(BF)
                    oring[h, pl.ds(opos, SEG), :] = o[0:SEG]
                    if par == 0:
                        lo = jnp.concatenate(
                            [oring[h, pl.ds(rpos, XR), :], o[mrow]], axis=0)
                    else:
                        lo = jnp.concatenate(
                            [o[mrow], oring[h, pl.ds(rpos, XR), :]], axis=0)
                    st['o', h] = lo

            def wo(g):
                lo = jnp.concatenate(
                    [st['o', h] for h in range(g * G, (g + 1) * G)], axis=1)
                for n in range(D // 128):
                    wt = wo_u32[n, pl.ds(g * G * 64, G * 64), :]
                    y = _dot(lo, pltpu.bitcast(wt, BF))
                    if g == 0:
                        acc_o[n] = y
                    elif g < NG - 1:
                        acc_o[n] += y
                    else:
                        st['a', n] = acc_o[n] + y

            for g in range(NG + 2):
                if g < NG:
                    proj(g, 0)
                if g == 0:
                    prev = 48 * j + XR * par - XR
                    prev = jnp.where(prev < 0, XR, prev)
                    finish_rows(att_buf[...], pl.multiple_of(prev, 8), XR)
                if 1 <= g <= NG:
                    pv(g - 1)
                if g < NG:
                    proj(g, 1)
                    proj(g, 2, 0, 2)
                    qk(g)
                    proj(g, 2, 2, 4)
                if 2 <= g:
                    wo(g - 2)
            lo_, hi_ = ((0, 24), (24, 32)) if par == 0 else ((8, 32), (0, 8))
            for n in range(D // 128):
                att_buf[:, n * 128:(n + 1) * 128] = st['a', n][lo_[0]:lo_[1]]
            mem_new = jnp.concatenate(
                [st['a', n][hi_[0]:hi_[1]] for n in range(D // 128)], axis=1)
            return mem_new.astype(BF)

        def dstep(j, mem):
            mem = step(mem, j, 0)
            return step(mem, j, 1)

        att_buf[...] = jnp.zeros((XR, D), F32)
        lax.fori_loop(0, NSEG // 2, dstep, mem0_ref[0])
        finish_rows(att_buf[...], XR * (NSEG - 1), XR)

        done = XR * NSEG
        cp_o0 = pltpu.make_async_copy(out_buf.at[pl.ds(0, done)],
                                      out_hbm.at[0, pl.ds(0, done)], fsem.at[3])
        cp_o0.start()

        def tail_rows(b, _):
            r = pl.multiple_of(done + 64 * b, 64)
            pos = pl.multiple_of(lax.rem(r, RING), 64)
            lo = jnp.concatenate(
                [oring[h, pl.ds(pos, 64), :] for h in range(H)], axis=1)
            att = jnp.concatenate(
                [_dot(lo, wo_all[n]) for n in range(D // 128)], axis=1)
            finish_rows(att, r, 64)
            return 0

        lax.fori_loop(0, (S - done) // 64, tail_rows, 0)

        ridx = lax.broadcasted_iota(jnp.int32, (S, 128), 0)
        rv = r_buf[...]
        m1 = jnp.max(rv)
        i1 = jnp.min(jnp.where(rv == m1, ridx, S))
        rv2 = jnp.where(ridx == i1, -jnp.inf, rv)
        m2 = jnp.max(rv2)
        i2 = jnp.min(jnp.where((rv2 == m2) & (ridx != i1), ridx, S))
        i1 = jnp.clip(i1, 0, S - 1)
        i2 = jnp.clip(i2, 0, S - 1)

        slab_i = lax.broadcasted_iota(jnp.int32, (16, D), 0)

        def get_row(i):
            b = pl.multiple_of((i // 16) * 16, 16)
            slab = x_buf[pl.ds(b, 16), :].astype(F32)
            return jnp.sum(jnp.where(slab_i == i - b, slab, 0.0), axis=0,
                           keepdims=True)

        x2s = jnp.where(slab_i == 0, get_row(i1),
                        jnp.where(slab_i == 1, get_row(i2), 0.0))
        h2s = (_ln(x2s) * cb1 + sb).astype(BF)

        for cp in ffn_copies:
            cp.wait()
        gu = []
        for n in range(F // 128):
            g = _dot(h2s, wg[n]).astype(BF).astype(F32)
            u = _dot(h2s, wu[n]).astype(BF).astype(F32)
            g = (g * jax.nn.sigmoid(g)).astype(BF).astype(F32)
            gu.append((g * u).astype(BF))
        gu = jnp.concatenate(gu, axis=1)
        y = jnp.concatenate([_dot(gu, wd[n]) for n in range(D // 128)], axis=1)
        rsel = jnp.where(slab_i[:, 0:1] == 0, m1, m2)
        y = y.astype(BF).astype(F32) * jax.nn.sigmoid(rsel)
        fixed = x2s + gb * (h2s.astype(F32) + y.astype(BF).astype(F32))

        cp_o0.wait()

        def put_row(i, row):
            b = pl.multiple_of((i // 16) * 16, 16)
            slab = out_buf[pl.ds(b, 16), :].astype(F32)
            out_buf[pl.ds(b, 16), :] = jnp.where(
                slab_i == i - b, row, slab).astype(BF)
            return b

        b1 = put_row(i1, fixed[0:1])
        b2 = put_row(i2, fixed[1:2])
        cp_o1 = pltpu.make_async_copy(out_buf.at[pl.ds(done, S - done)],
                                      out_hbm.at[0, pl.ds(done, S - done)],
                                      fsem.at[3])
        cp_o1.start()
        cp_o1.wait()
        for b in (b1, b2):
            cp = pltpu.make_async_copy(out_buf.at[pl.ds(b, 16)],
                                       out_hbm.at[0, pl.ds(b, 16)], fsem.at[3])
            cp.start()
            cp.wait()

    pl.run_scoped(
        main,
        pltpu.VMEM((F // 128, D, 128), BF),
        pltpu.VMEM((F // 128, D, 128), BF),
        pltpu.VMEM((D // 128, F, 128), BF),
        pltpu.SemaphoreType.DMA((4,)),
        pltpu.VMEM((D // 128, 32, 128), F32),
        pltpu.VMEM((XR, D), F32),
    )


@functools.partial(jax.jit, static_argnames=("A_seg_len",))
def pallas_adaLN_cond__memory_aug_recurrent_mem_tr__moe_arch_mod__prompt_kernel(
    A_x: jax.Array,
    A_mem0: jax.Array,
    A_Wq: jax.Array,
    A_Wk: jax.Array,
    A_Wv: jax.Array,
    A_Wo: jax.Array,
    A_seg_len: int,
    B_x: jax.Array,
    B_w_r: jax.Array,
    B_w_gate: jax.Array,
    B_w_up: jax.Array,
    B_w_down: jax.Array,
    c: jax.Array,
    w_mod: jax.Array,
):
    assert int(A_seg_len) == SEG
    assert A_x.shape == (1, S, D) and A_Wq.shape == (D, H, DH)
    vm = pl.BlockSpec(memory_space=pltpu.VMEM)
    hbm = pl.BlockSpec(memory_space=pl.ANY)
    return pl.pallas_call(
        _kernel,
        out_shape=jax.ShapeDtypeStruct((1, S, D), BF),
        in_specs=[vm, vm, vm] + [hbm] * 9,
        out_specs=hbm,
        scratch_shapes=[
            pltpu.VMEM((3 * H, D // 2, DH), jnp.uint32),
            pltpu.VMEM((D // 128, H * DH, 128), BF),
            pltpu.VMEM((S, D), BF),
            pltpu.VMEM((S, D), BF),
            pltpu.VMEM((H, RING, DH), BF),
            pltpu.VMEM((H, RING, DH), BF),
            pltpu.VMEM((H, RING, DH), BF),
            pltpu.VMEM((H, RING, DH), BF),
            pltpu.VMEM((S, D), BF),
            pltpu.VMEM((S, 128), F32),
            pltpu.VMEM((6, 8, D), F32),
            pltpu.SemaphoreType.DMA((3,)),
        ],
        compiler_params=pltpu.CompilerParams(
            vmem_limit_bytes=120 * 1024 * 1024),
    )(c, B_w_r, A_mem0, A_x, A_Wq, A_Wk, A_Wv,
      A_Wo.reshape(H * DH, D), B_w_gate, B_w_up, B_w_down, w_mod)
```

```python
import functools

import jax
import jax.numpy as jnp
from jax import lax
import jax.experimental.pallas as pl
import jax.experimental.pallas.tpu as pltpu

BF = jnp.bfloat16
F32 = jnp.float32

S = 2048
D = 1024
H = 32
DH = 128
NM = 8
SEG = 32
NSEG = S // SEG
F = 3584
R0 = 512
XR = 24
RING = 576
QOFF = 64
EPS = 1e-5
NEG = -1000000000.0
KC = 256
NKC = D // KC
TS = 17


def _dot(a, b):
    return jnp.dot(a, b, preferred_element_type=F32)


def _dot_t(a, b):
    return lax.dot_general(a, b, (((1,), (1,)), ((), ())),
                           preferred_element_type=F32)


def _ln(xf):
    m = jnp.mean(xf, axis=-1, keepdims=True)
    d = xf - m
    v = jnp.mean(d * d, axis=-1, keepdims=True)
    return d * lax.rsqrt(v + EPS)


def _kernel(c_ref, wr_ref, mem0_ref, x_hbm, wq_hbm, wk_hbm, wv_hbm, wo_hbm,
            wg_hbm, wu_hbm, wd_hbm, wmod_hbm, out_hbm,
            w_all, wo_all, x_buf, h_buf, ring_q, ring_k, ring_v, oring, out_buf, r_buf, mod_buf,
            sems):
    w_hbm = (wq_hbm, wk_hbm, wv_hbm)
    ring = (ring_q, ring_k, ring_v)
    scale = DH ** (-0.5)

    cp_x0 = pltpu.make_async_copy(x_hbm.at[0, pl.ds(0, R0)],
                                  x_buf.at[pl.ds(0, R0)], sems.at[0])
    cp_x1 = pltpu.make_async_copy(x_hbm.at[0, pl.ds(R0, S - R0)],
                                  x_buf.at[pl.ds(R0, S - R0)], sems.at[1])

    def cp_wo(n):
        c0 = pl.multiple_of(n * 128, 128)
        return pltpu.make_async_copy(wo_hbm.at[:, pl.ds(c0, 128)],
                                     wo_all.at[n], sems.at[2])

    def prologue(wm_buf, stage, tmp, acc, psem):
        cp_m0 = pltpu.make_async_copy(wmod_hbm.at[:, pl.ds(0, 2 * D)],
                                      wm_buf.at[:, pl.ds(0, 2 * D)], psem.at[3])

        def cp_m1(n):
            c0 = pl.multiple_of(2 * D + n * 512, 512)
            return pltpu.make_async_copy(wmod_hbm.at[:, pl.ds(c0, 512)],
                                         wm_buf.at[:, pl.ds(c0, 512)], psem.at[4])

        def chunk_copy(w, kc, slot):
            return pltpu.make_async_copy(
                w_hbm[w].at[pl.ds(kc * KC, KC)], stage.at[slot],
                psem.at[slot])

        chunk_copy(0, 0, 0).start()
        cp_m0.start()
        cp_x0.start()

        cf = c_ref[...].astype(F32)
        sc = (cf * jax.nn.sigmoid(cf)).astype(BF)
        sc16 = jnp.broadcast_to(sc, (16, D))

        def mod_cols(lo, hi):
            for j in range(lo, hi):
                m = _dot(sc16, wm_buf[:, j * D:(j + 1) * D])
                mod_buf[j] = m[0:8].astype(BF).astype(F32)

        def ln_rows(r, n):
            r = pl.multiple_of(r, 16)
            xf = x_buf[pl.ds(r, n), :].astype(F32)
            h_buf[pl.ds(r, n), :] = (_ln(xf) * (1.0 + mod_buf[1][0:1]) + mod_buf[0][0:1]).astype(BF)

        def ln_loop(i, _):
            ln_rows(i * 64, 64)
            return 0

        def unpack_stage(slot):
            for dc in range(KC // 16):
                v = stage[slot, pl.ds(dc * 16, 16)]
                u = pltpu.bitcast(v, jnp.uint32)
                for d in range(16):
                    tmp[pl.ds((dc * 16 + d) * TS, 16), :] = u[d]

        def relayout_pair(w, kc, hp):
            k0 = pl.multiple_of(kc * (KC // 2), KC // 2)
            a = tmp[pl.ds(hp, KC, stride=TS), :]
            lo = pltpu.bitcast(a << 16, F32).astype(BF)
            hi = pltpu.bitcast(a & jnp.uint32(0xFFFF0000), F32).astype(BF)
            w_all[w * H + 2 * hp, pl.ds(k0, KC // 2), :] = pltpu.bitcast(lo, jnp.uint32)
            w_all[w * H + 2 * hp + 1, pl.ds(k0, KC // 2), :] = pltpu.bitcast(hi, jnp.uint32)

        nchunk = NKC * 3

        def start_chunk(ci):
            for w in range(3):
                @pl.when((ci >= NKC * w) & (ci < NKC * w + NKC))
                def _():
                    kc = pl.multiple_of((ci - NKC * w) * KC, KC)
                    pltpu.make_async_copy(
                        w_hbm[w].at[pl.ds(kc, KC)], stage.at[ci % 3],
                        psem.at[ci % 3]).start()

        def wait_chunk(ci):
            chunk_copy(0, 0, ci % 3).wait()

        wait_chunk(0)
        chunk_copy(0, 1, 1).start()
        unpack_stage(0)
        for hp in range(H // 2):
            relayout_pair(0, 0, hp)
        cp_m0.wait()
        mod_cols(0, 2)

        chunk_copy(0, 2, 2).start()
        cp_x1.start()
        cp_x0.wait()
        lax.fori_loop(0, R0 // 64, ln_loop, 0)

        LNR = (S - R0) // (nchunk - NKC)

        def chunk_body(ci, with_ln):
            w, kc = ci // NKC, ci % NKC
            cn = jnp.minimum(ci + 1, nchunk - 1)
            start_chunk(ci + 3)
            if with_ln:
                cp_m1(ci - NKC).start()
                cp_wo(ci - NKC).start()

            @pl.when(ci + 1 < nchunk)
            def _():
                wait_chunk(ci + 1)

            k0 = pl.multiple_of(kc * KC, KC)
            lhs = h_buf[pl.ds(0, R0), pl.ds(k0, KC)]
            kw = pl.multiple_of(kc * (KC // 2), KC // 2)
            first = kc == 0
            hp_next = 0
            for h in range(H):
                y = _dot(lhs, pltpu.bitcast(w_all[w * H + h, pl.ds(kw, KC // 2), :], BF))
                acc[h] = jnp.where(first, y, acc[h] + y)
                if h == 3:
                    unpack_stage(cn % 3)
                if h >= 8 and h % 3 != 0:
                    relayout_pair(cn // NKC, cn % NKC, hp_next)
                    hp_next += 1
                if with_ln and h == 4:
                    ln_rows(R0 + (ci - NKC) * LNR, LNR)

            for wi in range(3):
                @pl.when(ci == NKC * wi + NKC - 1)
                def _():
                    def cvt(h, _):
                        ring[wi][h, pl.ds(QOFF, R0), :] = acc[h].astype(BF)
                        return 0
                    lax.fori_loop(0, H, cvt, 0, unroll=4)
            return 0

        acc[...] = jnp.zeros_like(acc)
        lax.fori_loop(0, NKC, lambda ci, _: chunk_body(ci, False), 0)
        cp_x1.wait()
        lax.fori_loop(NKC, nchunk, lambda ci, _: chunk_body(ci, True), 0)

        for n in range(8):
            cp_m1(n).wait()
        mod_cols(2, 6)
        for n in range(8):
            cp_wo(n).wait()

    pl.run_scoped(
        prologue,
        pltpu.VMEM((D, 6 * D), BF),
        pltpu.VMEM((3, KC, H, DH), BF),
        pltpu.VMEM((KC * TS, 128), jnp.uint32),
        pltpu.VMEM((H, R0, 128), F32),
        pltpu.SemaphoreType.DMA((5,)),
    )

    def main(wg, wu, wd, fsem, acc_o, att_buf, att2):
        wo_u32 = wo_all.bitcast(jnp.uint32)
        ffn_copies = []
        for n in range(F // 128):
            ffn_copies.append(pltpu.make_async_copy(
                wg_hbm.at[:, pl.ds(n * 128, 128)], wg.at[n], fsem.at[0]))
            ffn_copies.append(pltpu.make_async_copy(
                wu_hbm.at[:, pl.ds(n * 128, 128)], wu.at[n], fsem.at[1]))
        for n in range(D // 128):
            ffn_copies.append(pltpu.make_async_copy(
                wd_hbm.at[:, pl.ds(n * 128, 128)], wd.at[n], fsem.at[2]))
        for cp in ffn_copies:
            cp.start()

        ga = mod_buf[2][0:1]
        sb = mod_buf[3][0:1]
        cb1 = 1.0 + mod_buf[4][0:1]
        gb = mod_buf[5][0:1]
        wr = wr_ref[...].astype(F32).reshape(1, D)

        def finish_rows(att, r, n):
            rows = pl.ds(r, n)
            x2 = (x_buf[rows, :].astype(F32)
                  + ga * att.astype(BF).astype(F32)).astype(BF)
            x_buf[rows, :] = x2
            x2f = x2.astype(F32)
            h2 = (_ln(x2f) * cb1 + sb).astype(BF).astype(F32)
            out_buf[rows, :] = (x2f + gb * h2).astype(BF)
            rr = jnp.sum(h2 * wr, axis=-1, keepdims=True)
            rr = rr.astype(BF).astype(F32)
            r_buf[rows, :] = jnp.broadcast_to(rr, (n, 128))

        def attn_mask(par):
            qi = lax.broadcasted_iota(jnp.int32, (48, 48), 0)
            ki = lax.broadcasted_iota(jnp.int32, (48, 48), 1)
            mlo = 40 if par == 0 else 32
            kmem = (ki >= mlo) & (ki < mlo + NM)
            kx = ki < SEG
            return kmem | (kx & ((qi >= SEG) | (qi >= ki)))

        def step(mem, j, par):
            s = 2 * j + par
            xr = pl.multiple_of(R0 + 48 * j + XR * par, 8)
            hx = h_buf[pl.ds(xr, XR), :]
            lhs = (jnp.concatenate([hx, mem], axis=0) if par == 0
                   else jnp.concatenate([mem, hx], axis=0))
            wbase = lax.rem(R0 + QOFF + 48 * j, RING)
            wpos = pl.multiple_of(wbase + XR * par, 8)
            spos = pl.multiple_of(lax.rem(SEG * s + QOFF, RING), SEG)
            opos = pl.multiple_of(lax.rem(SEG * s, RING), SEG)
            obase = lax.rem(48 * j, RING)
            rpos = pl.multiple_of(obase + XR * par, 8)
            mask = attn_mask(par)
            mrow = (slice(40, 48) if par == 0 else slice(32, 40))

            G = 4
            NG = H // G
            st = {}

            def proj(g, w, lo=0, hi=G):
                for h in range(g * G + lo, g * G + hi):
                    y = _dot(lhs, pltpu.bitcast(w_all[w * H + h], BF)).astype(BF)
                    if par == 0:
                        ring[w][h, pl.ds(wpos, XR), :] = y[0:24]
                        st[w, h] = y[16:32]
                    else:
                        ring[w][h, pl.ds(wpos, XR), :] = y[8:32]
                        st[w, h] = y[0:16]

            def seg(w, h):
                return jnp.concatenate(
                    [ring[w][h, pl.ds(spos, SEG), :], st[w, h]], axis=0)

            def qk(g):
                for h in range(g * G, (g + 1) * G):
                    sc = _dot_t(seg(0, h), seg(1, h)) * scale
                    sc = jnp.where(mask, sc, NEG)
                    mx = jnp.max(sc, axis=-1, keepdims=True)
                    e = jnp.exp(sc - mx)
                    st['p', h] = e.astype(BF)
                    den = jnp.sum(e, axis=-1, keepdims=True)
                    r = pl.reciprocal(den, approx=True)
                    st['r', h] = r * (2.0 - den * r)

            def pv(g):
                for h in range(g * G, (g + 1) * G):
                    o = (_dot(st['p', h], seg(2, h)) * st['r', h]).astype(BF)
                    oring[h, pl.ds(opos, SEG), :] = o[0:SEG]
                    if par == 0:
                        lo = jnp.concatenate(
                            [oring[h, pl.ds(rpos, XR), :], o[mrow]], axis=0)
                    else:
                        lo = jnp.concatenate(
                            [o[mrow], oring[h, pl.ds(rpos, XR), :]], axis=0)
                    st['o', h] = lo

            def wo(g):
                lo = jnp.concatenate(
                    [st['o', h] for h in range(g * G, (g + 1) * G)], axis=1)
                for n in range(D // 128):
                    wt = wo_u32[n, pl.ds(g * G * 64, G * 64), :]
                    y = _dot(lo, pltpu.bitcast(wt, BF))
                    if g == 0:
                        acc_o[n] = y
                    elif g < NG - 1:
                        acc_o[n] += y
                    else:
                        st['a', n] = acc_o[n] + y

            for g in range(NG + 2):
                if g < NG:
                    proj(g, 0)
                if g == 0:
                    prev = 48 * j + XR * par - XR
                    prev = jnp.where(prev < 0, XR, prev)
                    finish_rows(att_buf[...], pl.multiple_of(prev, 8), XR)
                if g < NG:
                    proj(g, 1)
                if 1 <= g <= NG:
                    pv(g - 1)
                if g < NG:
                    proj(g, 2, 0, 2)
                    qk(g)
                    proj(g, 2, 2, 4)
                if 2 <= g:
                    wo(g - 2)
            lo_, hi_ = ((0, 24), (24, 32)) if par == 0 else ((8, 32), (0, 8))
            for n in range(D // 128):
                att_buf[:, n * 128:(n + 1) * 128] = st['a', n][lo_[0]:lo_[1]]
            mem_new = jnp.concatenate(
                [st['a', n][hi_[0]:hi_[1]] for n in range(D // 128)], axis=1)
            return mem_new.astype(BF)

        def dstep(j, mem):
            mem = step(mem, j, 0)
            return step(mem, j, 1)

        att_buf[...] = jnp.zeros((XR, D), F32)
        lax.fori_loop(0, NSEG // 2, dstep, mem0_ref[0])
        finish_rows(att_buf[...], XR * (NSEG - 1), XR)

        done = XR * NSEG
        cp_o0 = pltpu.make_async_copy(out_buf.at[pl.ds(0, done)],
                                      out_hbm.at[0, pl.ds(0, done)], fsem.at[3])
        cp_o0.start()

        def tail_rows(b, _):
            r = pl.multiple_of(done + 64 * b, 64)
            pos = pl.multiple_of(lax.rem(r, RING), 64)
            lo = jnp.concatenate(
                [oring[h, pl.ds(pos, 64), :] for h in range(H)], axis=1)
            for n in range(D // 128):
                att2[b % 2, :, n * 128:(n + 1) * 128] = _dot(lo, wo_all[n])
                if n == 0:
                    finish_rows(att2[1 - b % 2], pl.multiple_of(r - 64 * jnp.minimum(b, 1), 64), 64)
            return 0

        att2[1] = jnp.zeros((64, D), F32)
        lax.fori_loop(0, (S - done) // 64, tail_rows, 0)
        finish_rows(att2[1], S - 64, 64)

        ridx = lax.broadcasted_iota(jnp.int32, (S, 128), 0)
        rv = r_buf[...]
        m1 = jnp.max(rv)
        i1 = jnp.min(jnp.where(rv == m1, ridx, S))
        rv2 = jnp.where(ridx == i1, -jnp.inf, rv)
        m2 = jnp.max(rv2)
        i2 = jnp.min(jnp.where((rv2 == m2) & (ridx != i1), ridx, S))
        i1 = jnp.clip(i1, 0, S - 1)
        i2 = jnp.clip(i2, 0, S - 1)

        slab_i = lax.broadcasted_iota(jnp.int32, (16, D), 0)

        def get_row(i):
            b = pl.multiple_of((i // 16) * 16, 16)
            slab = x_buf[pl.ds(b, 16), :].astype(F32)
            return jnp.sum(jnp.where(slab_i == i - b, slab, 0.0), axis=0,
                           keepdims=True)

        x2s = jnp.where(slab_i == 0, get_row(i1),
                        jnp.where(slab_i == 1, get_row(i2), 0.0))
        h2s = (_ln(x2s) * cb1 + sb).astype(BF)

        for cp in ffn_copies:
            cp.wait()
        gu = []
        for n in range(F // 128):
            g = _dot(h2s, wg[n]).astype(BF).astype(F32)
            u = _dot(h2s, wu[n]).astype(BF).astype(F32)
            g = (g * jax.nn.sigmoid(g)).astype(BF).astype(F32)
            gu.append((g * u).astype(BF))
        gu = jnp.concatenate(gu, axis=1)
        y = jnp.concatenate([_dot(gu, wd[n]) for n in range(D // 128)], axis=1)
        rsel = jnp.where(slab_i[:, 0:1] == 0, m1, m2)
        y = y.astype(BF).astype(F32) * jax.nn.sigmoid(rsel)
        fixed = x2s + gb * (h2s.astype(F32) + y.astype(BF).astype(F32))

        cp_o0.wait()

        def put_row(i, row):
            b = pl.multiple_of((i // 16) * 16, 16)
            slab = out_buf[pl.ds(b, 16), :].astype(F32)
            out_buf[pl.ds(b, 16), :] = jnp.where(
                slab_i == i - b, row, slab).astype(BF)
            return b

        b1 = put_row(i1, fixed[0:1])
        b2 = put_row(i2, fixed[1:2])
        cp_o1 = pltpu.make_async_copy(out_buf.at[pl.ds(done, S - done)],
                                      out_hbm.at[0, pl.ds(done, S - done)],
                                      fsem.at[3])
        cp_o1.start()
        cp_o1.wait()
        for b in (b1, b2):
            cp = pltpu.make_async_copy(out_buf.at[pl.ds(b, 16)],
                                       out_hbm.at[0, pl.ds(b, 16)], fsem.at[3])
            cp.start()
            cp.wait()

    pl.run_scoped(
        main,
        pltpu.VMEM((F // 128, D, 128), BF),
        pltpu.VMEM((F // 128, D, 128), BF),
        pltpu.VMEM((D // 128, F, 128), BF),
        pltpu.SemaphoreType.DMA((4,)),
        pltpu.VMEM((D // 128, 32, 128), F32),
        pltpu.VMEM((XR, D), F32),
        pltpu.VMEM((2, 64, D), F32),
    )


@functools.partial(jax.jit, static_argnames=("A_seg_len",))
def pallas_adaLN_cond__memory_aug_recurrent_mem_tr__moe_arch_mod__prompt_kernel(
    A_x: jax.Array,
    A_mem0: jax.Array,
    A_Wq: jax.Array,
    A_Wk: jax.Array,
    A_Wv: jax.Array,
    A_Wo: jax.Array,
    A_seg_len: int,
    B_x: jax.Array,
    B_w_r: jax.Array,
    B_w_gate: jax.Array,
    B_w_up: jax.Array,
    B_w_down: jax.Array,
    c: jax.Array,
    w_mod: jax.Array,
):
    assert int(A_seg_len) == SEG
    assert A_x.shape == (1, S, D) and A_Wq.shape == (D, H, DH)
    vm = pl.BlockSpec(memory_space=pltpu.VMEM)
    hbm = pl.BlockSpec(memory_space=pl.ANY)
    return pl.pallas_call(
        _kernel,
        out_shape=jax.ShapeDtypeStruct((1, S, D), BF),
        in_specs=[vm, vm, vm] + [hbm] * 9,
        out_specs=hbm,
        scratch_shapes=[
            pltpu.VMEM((3 * H, D // 2, DH), jnp.uint32),
            pltpu.VMEM((D // 128, H * DH, 128), BF),
            pltpu.VMEM((S, D), BF),
            pltpu.VMEM((S, D), BF),
            pltpu.VMEM((H, RING, DH), BF),
            pltpu.VMEM((H, RING, DH), BF),
            pltpu.VMEM((H, RING, DH), BF),
            pltpu.VMEM((H, RING, DH), BF),
            pltpu.VMEM((S, D), BF),
            pltpu.VMEM((S, 128), F32),
            pltpu.VMEM((6, 8, D), F32),
            pltpu.SemaphoreType.DMA((3,)),
        ],
        compiler_params=pltpu.CompilerParams(
            vmem_limit_bytes=120 * 1024 * 1024),
    )(c, B_w_r, A_mem0, A_x, A_Wq, A_Wk, A_Wv,
      A_Wo.reshape(H * DH, D), B_w_gate, B_w_up, B_w_down, w_mod)
```
